```python
import os as _os
_os.environ.setdefault('JAX_PLATFORMS', 'cpu')
import jax
import jax.numpy as jnp

def _softmax(x, axis=-1):
    return jax.nn.softmax(x, axis=axis)

def _gelu(x):
    return jax.nn.gelu(x, approximate=True)

def _silu(x):
    return jax.nn.silu(x)

def _sigmoid(x):
    return jax.nn.sigmoid(x)

def _layernorm(x, axis=-1, eps=1e-05):
    m = jnp.mean(x, axis=axis, keepdims=True)
    v = jnp.var(x, axis=axis, keepdims=True)
    return (x - m) / jnp.sqrt(v + eps)

def _scatter_add(tgt, idx, src, axis=0):
    return tgt.at[idx].add(src)

def _segment_sum(src, seg, n):
    return jax.ops.segment_sum(src, seg, n)

class _Rng:

    def __init__(self, key):
        self._k = key

    def _next(self):
        self._k, sub = jax.random.split(self._k)
        return sub

    def normal(self, shape):
        return jax.random.normal(self._next(), shape, dtype=jnp.bfloat16)

    def randint(self, lo, hi, shape):
        return jax.random.randint(self._next(), shape, lo, hi, dtype=jnp.int32)

    def uniform(self, shape, lo=0.0, hi=1.0):
        return jax.random.uniform(self._next(), shape, jnp.bfloat16, lo, hi)

    def permutation(self, n):
        return jax.random.permutation(self._next(), n)
kernel_name = 'gated_mix__sliding_block__memory_aug_recurrent_mem_tr__prompt'

def setup_inputs():
    _rng = _Rng(jax.random.key(int.from_bytes(__import__("os").urandom(4), "little")))
    _w = lambda a: (lambda t: t.astype(jnp.bfloat16) if jnp.issubdtype(t.dtype, jnp.floating) else t)(jnp.asarray(a))

    def _A_setup():
        B, S, D = (1, 2048, 448)
        return {'x': _w((lambda *s: _rng.normal(s) * 0.05)(B, S, D)), 'wqkv': _w((lambda *s: _rng.normal(s) * 0.8)(D, 3 * D)), 'wo': _w((lambda *s: _rng.normal(s) * 0.05)(D, D))}
    _A_in = _A_setup()

    def _B_setup():
        B, S, Dm = (1, 2048, 448)
        H, Dh = (16, 256)
        M, seg = (8, 32)
        seg = min(seg, S)
        S = S // seg * seg
        return {'x': _w((lambda *s: _rng.normal(s) * 0.05)(B, S, Dm)), 'mem0': _w((lambda *s: _rng.normal(s) * 0.8)(B, M, Dm)), 'Wq': _w((lambda *s: _rng.normal(s) * 3.2)(Dm, H, Dh) * Dm ** (-0.5)), 'Wk': _w((lambda *s: _rng.normal(s) * 3.2)(Dm, H, Dh) * Dm ** (-0.5)), 'Wv': _w((lambda *s: _rng.normal(s) * 0.8)(Dm, H, Dh) * Dm ** (-0.5)), 'Wo': _w((lambda *s: _rng.normal(s) * 0.8)(H, Dh, Dm) * (H * Dh) ** (-0.5)), 'seg_len': seg}
    _B_in = _B_setup()
    return {'A_x': _A_in['x'], 'A_wqkv': _A_in['wqkv'], 'A_wo': _A_in['wo'], 'B_x': _B_in['x'], 'B_mem0': _B_in['mem0'], 'B_Wq': _B_in['Wq'], 'B_Wk': _B_in['Wk'], 'B_Wv': _B_in['Wv'], 'B_Wo': _B_in['Wo'], 'B_seg_len': _B_in['seg_len'], 'gate_w': _w((lambda *s: _rng.normal(s) * 0.05)(448) * 16.0)}

def reference(A_x, A_wqkv, A_wo, B_x, B_mem0, B_Wq, B_Wk, B_Wv, B_Wo, B_seg_len, gate_w):

    def _A_ref(x, wqkv, wo):
        B, S, D = x.shape
        H = 16
        Dh = D // H
        W = 256
        qkv = (lambda x, *d: x.transpose(*d))((x @ wqkv).reshape(B, S, 3, H, Dh), 2, 0, 3, 1, 4)
        q, k, v = (qkv[0], qkv[1], qkv[2])
        scores = jnp.einsum('bhqd,bhkd->bhqk', q, k) * Dh ** (-0.5)
        idx = jnp.arange(S)
        mask = (idx[:, None] - idx[None, :] >= 0) & (idx[:, None] - idx[None, :] < W)
        scores = jnp.where(mask[None, None], scores, -1000000000.0)
        p = _softmax(scores, axis=-1)
        o = jnp.einsum('bhqk,bhkd->bhqd', p, v)
        return (lambda x, *d: x.transpose(*d))(o, 0, 2, 1, 3).reshape(B, S, D) @ wo

    def _B_ref(x, mem0, Wq, Wk, Wv, Wo, seg_len):
        B, S, Dm = x.shape
        H, Dh = (Wq.shape[1], Wq.shape[2])
        M = mem0.shape[1]
        scale = Dh ** (-0.5)
        n_seg = S // seg_len
        L = M + seg_len
        idx = jnp.arange(L)
        mask = (idx[:, None] < M) | (idx[:, None] >= idx[None, :])
        mem = mem0
        outs = []
        for s in range(n_seg):
            xs = x[:, s * seg_len:(s + 1) * seg_len, :].copy()
            h = jnp.concatenate([mem, xs], axis=1)
            q = jnp.einsum('btd,dhe->bhte', h, Wq)
            k = jnp.einsum('btd,dhe->bhte', h, Wk)
            v = jnp.einsum('btd,dhe->bhte', h, Wv)
            scores = jnp.einsum('bhqe,bhke->bhqk', q, k) * scale
            scores = jnp.where(mask[None, None], scores, -1000000000.0)
            p = _softmax(scores, axis=-1)
            o = jnp.einsum('bhqk,bhke->bhqe', p, v)
            o = jnp.einsum('bhte,hed->btd', o, Wo)
            mem = o[:, :M, :].copy()
            outs.append(o[:, M:, :])
        return jnp.concatenate(outs, axis=1)
    x = A_x
    g = _sigmoid((x * gate_w).sum(-1, keepdims=True))
    a = _A_ref(x, A_wqkv, A_wo)
    b = _B_ref(x, B_mem0, B_Wq, B_Wk, B_Wv, B_Wo, B_seg_len)
    return g * a + (1 - g) * b
```

```python
import functools
import math

import jax
import jax.numpy as jnp
from jax import lax
import jax.experimental.pallas as pl
import jax.experimental.pallas.tpu as pltpu

F32 = jnp.float32
BF16 = jnp.bfloat16

LANES = 128
A_HEADS = 16
A_WINDOW = 256
A_GROUP = 4
MASK_VALUE = -1e9
LOG2E = math.log2(math.e)

_NN = (((1,), (0,)), ((), ()))
_NT = (((1,), (1,)), ((), ()))


def _dot(a, b, dims=_NN):
    return lax.dot_general(a, b, dims, preferred_element_type=F32)


def _group8_allreduce(x, op):
    lane = lax.broadcasted_iota(jnp.int32, x.shape, 1)
    for k in (1, 2, 4):
        partner = jnp.where((lane & k) != 0,
                            pltpu.roll(x, k, 1), pltpu.roll(x, LANES - k, 1))
        x = op(x, partner)
    return x


def _kernel(xt_hbm, wqkv_hbm, awo_hbm, mem0_hbm, wq_hbm, wk_hbm, wv_hbm, wot_hbm, gw_hbm,
            out_hbm,
            xt_v, wqkv_v, awo_v, mem0_v, gw_v, wq_v, wk_v, wv_v, wot_v,
            wqkvt_v, awot_v, x_v, qt_v, k_v, vt_v, gate_v, w_v,
            zs_v, us_v, p_v, ot_v, b_v, out_v, in_sem, out_sem,
            *, S, D, H, DH, M, SEG):
    L = M + SEG
    NG = L // 8
    DF = D // LANES
    DR = D - DF * LANES
    DP = (DF + 1) * LANES
    NQB = S // LANES
    SPB = LANES // SEG
    ADH = D // A_HEADS
    AGW = A_GROUP * ADH
    NAG = A_HEADS // A_GROUP
    WB = A_WINDOW // LANES
    HW = H * D
    XC = 512

    copies = {}

    def fetch(name, src, dst):
        copies[name] = pltpu.make_async_copy(src, dst, in_sem.at[len(copies)])
        copies[name].start()

    fetch("wqkv", wqkv_hbm, wqkv_v)
    fetch("gw", gw_hbm, gw_v)
    for c in range(S // XC):
        fetch(("x", c), xt_hbm.at[:, pl.ds(c * XC, XC)], xt_v.at[:, pl.ds(c * XC, XC)])
    fetch("awo", awo_hbm, awo_v)
    fetch("mem0", mem0_hbm, mem0_v)
    for name, src, dst in (("wk", wk_hbm, wk_v), ("wq", wq_hbm, wq_v), ("wv", wv_hbm, wv_v)):
        for c in range(DH // LANES):
            fetch((name, c), src.at[:, pl.ds(c * LANES, LANES)], dst.at[c])
    fetch("wot", wot_hbm, wot_v)

    lane = lax.broadcasted_iota(jnp.int32, (A_WINDOW, LANES), 1)
    for g in range(NAG):
        k_v[g, 0:A_WINDOW, :] = jnp.where(lane == AGW, MASK_VALUE, 0.0).astype(BF16)
        for kb in range(WB):
            vt_v[g, kb] = jnp.zeros((AGW, LANES), F32)

    copies["wqkv"].wait()
    for c in range(0, 3 * D, LANES):
        n = min(LANES, 3 * D - c)
        wqkvt_v[c:c + n, :] = wqkv_v[:, c:c + n].T
    copies["gw"].wait()
    wqkvt_v[3 * D:3 * D + 16, :] = jnp.broadcast_to(gw_v[...].astype(F32), (16, D)).astype(BF16)

    q_scale = ADH ** -0.5 * LOG2E
    for c in range(S // XC):
        copies["x", c].wait()
        xt = xt_v[:, c * XC:(c + 1) * XC]
        r = _dot(wqkvt_v[...], xt)
        for t in range(XC // LANES):
            qb = c * (XC // LANES) + t
            cols = slice(t * LANES, (t + 1) * LANES)
            for g in range(NAG):
                rows = g * AGW
                qt_v[qb, g] = (r[rows:rows + AGW, cols] * q_scale).astype(BF16)
                kt = jnp.concatenate(
                    [r[D + rows:D + rows + AGW, cols], jnp.zeros((LANES - AGW, LANES), F32)], 0)
                k_v[g, A_WINDOW + qb * LANES:A_WINDOW + (qb + 1) * LANES, :] = kt.T.astype(BF16)
                vt_v[g, WB + qb] = r[2 * D + rows:2 * D + rows + AGW, cols]
            gate_v[qb] = jax.nn.sigmoid(r[3 * D:3 * D + 8, cols])
        for j in range(DF):
            x_v[c * XC:(c + 1) * XC, j * LANES:(j + 1) * LANES] = xt[j * LANES:(j + 1) * LANES].T
        x_v[c * XC:(c + 1) * XC, DF * LANES:] = jnp.concatenate([xt[DF * LANES:]] * 2, 0).T

    copies["awo"].wait()
    for g in range(NAG):
        blk = jnp.concatenate(
            [awo_v[g * AGW:(g + 1) * AGW, :], jnp.zeros((LANES - AGW, D), BF16)], 0)
        awot_v[0:D, g * LANES:(g + 1) * LANES] = blk.T
    awot_v[D:, :] = jnp.zeros((DP - D, NAG * LANES), BF16)

    def head_pair(ref, p):
        words = ref.bitcast(jnp.uint32)
        w = jnp.concatenate(
            [words[c, pl.ds(p, D, stride=H // 2), :] for c in range(DH // LANES)], 1)
        return (pltpu.bitcast(w << 16, F32),
                pltpu.bitcast(w & jnp.uint32(0xFFFF0000), F32))

    def fold(p, lhs, rhs, base, scale):
        rem = None
        for e in range(2):
            r = _dot(lhs[e], rhs[e][:DF * LANES], _NT) * scale
            for j in range(DF):
                col = base + (j * H + 2 * p + e) * LANES
                w_v[:, col:col + LANES] = r[:, j * LANES:(j + 1) * LANES].astype(BF16)
            zero = jnp.zeros((DR, DH), BF16)
            tail = rhs[e][DF * LANES:]
            part = _dot(lhs[e], jnp.concatenate([zero, tail] if e else [tail, zero], 0), _NT)
            rem = part if rem is None else rem + part
        col = base + (DF * H + p) * LANES
        w_v[:, col:col + LANES] = (rem * scale).astype(BF16)

    for name in ("wk", "wq"):
        for c in range(DH // LANES):
            copies[name, c].wait()

    for p in range(H // 2):
        fold(p, head_pair(wk_v, p), [w.astype(BF16) for w in head_pair(wq_v, p)],
             0, DH ** -0.5 * LOG2E)

    for c in range(DH // LANES):
        copies["wv", c].wait()
    copies["wot"].wait()

    for p in range(H // 2):
        fold(p, head_pair(wv_v, p), [wot_v[2 * p], wot_v[2 * p + 1]], HW, 1.0)

    def a_scores(qb, g):
        kwin = k_v[g, pl.ds(pl.multiple_of(qb * LANES, LANES), A_WINDOW + LANES), :]
        q = qt_v[qb, g]
        row = lax.broadcasted_iota(jnp.int32, (AGW, LANES), 0)
        bias_row = jnp.where(
            lax.broadcasted_iota(jnp.int32, (LANES - AGW, LANES), 0) == 0, 1.0, 0.0).astype(BF16)
        qs = []
        for j in range(A_GROUP):
            keep = (row >= j * ADH) & (row < (j + 1) * ADH)
            qs.append(jnp.concatenate(
                [jnp.where(keep, q.astype(F32), 0.0).astype(BF16), bias_row], 0))
        s = _dot(kwin, jnp.concatenate(qs, 1))
        old = (lax.broadcasted_iota(jnp.int32, (LANES, LANES), 1)
               < lax.broadcasted_iota(jnp.int32, (LANES, LANES), 0))
        inv = []
        for j in range(A_GROUP):
            sj = s[:, j * LANES:(j + 1) * LANES]
            edge = jnp.where(old, sj[:LANES], sj[A_WINDOW:])
            mid = sj[LANES:A_WINDOW]
            m = jnp.maximum(jnp.max(edge, 0, keepdims=True), jnp.max(mid, 0, keepdims=True))
            edge = jnp.exp2(edge - m)
            mid = jnp.exp2(mid - m)
            inv.append(1.0 / (jnp.sum(edge, 0, keepdims=True) + jnp.sum(mid, 0, keepdims=True)))
            p_v[j, 0:LANES] = jnp.where(old, edge, 0.0).astype(BF16)
            p_v[j, LANES:A_WINDOW] = mid.astype(BF16)
            p_v[j, A_WINDOW:] = jnp.where(old, 0.0, edge).astype(BF16)
        return inv

    def a_values(qb, g, slot, inv):
        vwin = jnp.concatenate([vt_v[g, qb + kb] for kb in range(WB + 1)], 1)
        o = []
        for j in range(A_GROUP):
            lo, hi = j * ADH // 8 * 8, -(-(j + 1) * ADH // 8) * 8
            o.append((lo, hi, _dot(vwin[lo:hi], p_v[j]) * inv[j]))
        sub = lax.broadcasted_iota(jnp.int32, (8, LANES), 0)
        tiles = []
        for r in range(0, AGW, 8):
            own = [(j, oj[r - lo:r - lo + 8]) for j, (lo, hi, oj) in enumerate(o) if lo <= r < hi]
            tile = own[-1][1]
            if len(own) == 2:
                tile = jnp.where(sub < own[1][0] * ADH - r, own[0][1], tile)
            tiles.append(tile)
        tiles.append(jnp.zeros((LANES - AGW, LANES), F32))
        ot_v[slot, g * LANES:(g + 1) * LANES, :] = jnp.concatenate(tiles, 0).astype(BF16)

    def mix(qb, slot, j):
        n = LANES if j < DF else DR
        a = _dot(awot_v[j * LANES:j * LANES + n, :], ot_v[slot])
        b = b_v[slot, :, j * LANES:(j + 1) * LANES].T
        if j == DF:
            b = b[:DR] + b[DR:]
        gate = gate_v[qb][0:1]
        out_v[qb, j * LANES:j * LANES + n, :] = (gate * a + (1.0 - gate) * b).astype(BF16)

    def project(h, base, dst, js):
        low = lax.broadcasted_iota(jnp.int32, (8, LANES), 1) < DR
        for j in js:
            width = (H if j < DF else H // 2) * LANES
            r = _dot(h, w_v[:, base + j * H * LANES:base + j * H * LANES + width])
            for g in range(NG):
                rows = r[g * 8:(g + 1) * 8]
                if j < DF:
                    tiles = [rows[:, n * LANES:(n + 1) * LANES] for n in range(H)]
                else:
                    tiles = []
                    for n in range(H // 2):
                        t = rows[:, n * LANES:(n + 1) * LANES]
                        tiles += [jnp.where(low, t, 0.0), jnp.where(low, 0.0, t)]
                dst[g * LANES:(g + 1) * LANES, j * LANES:(j + 1) * LANES] = (
                    jnp.concatenate(tiles, 0).astype(BF16))

    def b_softmax(s):
        causal = ((lax.broadcasted_iota(jnp.int32, (8, LANES), 1) & 7)
                  <= lax.broadcasted_iota(jnp.int32, (8, LANES), 0))
        tiles = []
        for i in range(NG):
            row = [s[i * 8:(i + 1) * 8, g * LANES:(g + 1) * LANES]
                   for g in range(NG if i == 0 else i + 1)]
            if i:
                row[i] = jnp.where(causal, row[i], MASK_VALUE)
            tiles.append(row)
        m = jnp.concatenate([functools.reduce(jnp.maximum, row) for row in tiles], 0)
        m = _group8_allreduce(m, jnp.maximum)
        tiles = [[jnp.exp2(t - m[i * 8:(i + 1) * 8]) for t in row] for i, row in enumerate(tiles)]
        z = jnp.concatenate([functools.reduce(jnp.add, row) for row in tiles], 0)
        z = 1.0 / _group8_allreduce(z, jnp.add)
        zero = jnp.zeros((8, LANES), F32)
        return jnp.concatenate(
            [jnp.concatenate([t * z[i * 8:(i + 1) * 8] for t in row]
                             + [zero] * (NG - len(row)), 1)
             for i, row in enumerate(tiles)], 0)

    def out_copy(qb):
        return pltpu.make_async_copy(
            out_v.at[qb], out_hbm.at[:, pl.ds(pl.multiple_of(qb * LANES, LANES), LANES)], out_sem)

    copies["mem0"].wait()
    mem0 = jnp.concatenate([mem0_v[...].astype(F32), jnp.zeros((M, DP - D), F32)], 1)
    ot_v[1] = jnp.zeros(ot_v.shape[1:], BF16)
    b_v[1] = jnp.zeros(b_v.shape[1:], F32)

    def block(qb, mem):
        slot = qb % 2
        prev = jnp.maximum(qb - 1, 0)
        for t in range(SPB):
            tail = mem[:, DF * LANES:]
            mem = jnp.concatenate([mem[:, :DF * LANES], tail + pltpu.roll(tail, DR, 1)], 1)
            xs = x_v[pl.ds(pl.multiple_of(qb * LANES + t * SEG, SEG), SEG), :]
            h = jnp.concatenate([mem, xs.astype(F32)], 0)

            inv = a_scores(qb, t)
            project(h[:, :D], 0, zs_v, range(DF + 1))
            project(h[:, :D], HW, us_v, range(1))
            p = b_softmax(_dot(h, zs_v[...], _NT))
            project(h[:, :D], HW, us_v, range(1, DF + 1))
            a_values(qb, t, slot, inv)
            mix(prev, 1 - slot, t)
            o = _dot(p, us_v[...])
            b_v[slot, t * SEG:(t + 1) * SEG, :] = o[M:]
            mem = o[:M]

        @pl.when(qb > 0)
        def _():
            out_copy(prev).start()

        return mem

    lax.fori_loop(0, NQB, block, mem0)

    for j in range(DF + 1):
        mix(NQB - 1, (NQB - 1) % 2, j)
    out_copy(NQB - 1).start()
    for qb in range(NQB):
        out_copy(qb).wait()


@functools.partial(jax.jit, static_argnames=("B_seg_len",))
def pallas_gated_mix__sliding_block__memory_aug_recurrent_mem_tr__prompt_kernel(
    A_x, A_wqkv, A_wo, B_x, B_mem0, B_Wq, B_Wk, B_Wv, B_Wo, B_seg_len, gate_w,
):
    del B_x
    batch, S, D = A_x.shape
    _, H, DH = B_Wq.shape
    M, SEG = B_mem0.shape[1], int(B_seg_len)
    L = M + SEG
    DP = -(-D // LANES) * LANES
    NQB = S // LANES
    AGW = A_GROUP * D // A_HEADS
    NAG = A_HEADS // A_GROUP
    assert batch == 1 and M == 8 and H * 8 == LANES and DP - D == LANES // 2
    assert LANES // SEG == NAG == DP // LANES and SEG % 16 == 0

    hbm = pl.BlockSpec(memory_space=pltpu.HBM)
    vmem = pltpu.VMEM
    out_t = pl.pallas_call(
        functools.partial(_kernel, S=S, D=D, H=H, DH=DH, M=M, SEG=SEG),
        out_shape=jax.ShapeDtypeStruct((D, S), A_x.dtype),
        in_specs=[hbm] * 9,
        out_specs=hbm,
        scratch_shapes=[
            vmem((D, S), BF16),
            vmem((D, 3 * D), BF16),
            vmem((D, D), BF16),
            vmem((M, D), BF16),
            vmem((1, D), BF16),
            vmem((DH // LANES, D * H, LANES), BF16),
            vmem((DH // LANES, D * H, LANES), BF16),
            vmem((DH // LANES, D * H, LANES), BF16),
            vmem((H, D, DH), BF16),
            vmem((3 * D + 16, D), BF16),
            vmem((DP, NAG * LANES), BF16),
            vmem((S, DP), BF16),
            vmem((NQB, NAG, AGW, LANES), BF16),
            vmem((NAG, A_WINDOW + S, LANES), BF16),
            vmem((NAG, A_WINDOW // LANES + NQB, AGW, LANES), F32),
            vmem((NQB, 8, LANES), F32),
            vmem((D, 2 * H * D), BF16),
            vmem((H * L, DP), BF16),
            vmem((H * L, DP), BF16),
            vmem((A_GROUP, A_WINDOW + LANES, LANES), BF16),
            vmem((2, NAG * LANES, LANES), BF16),
            vmem((2, LANES, DP), F32),
            vmem((NQB, D, LANES), BF16),
            pltpu.SemaphoreType.DMA((16,)),
            pltpu.SemaphoreType.DMA(()),
        ],
        compiler_params=pltpu.CompilerParams(vmem_limit_bytes=100 * 1024 * 1024),
    )(
        A_x[0].T, A_wqkv, A_wo, B_mem0[0],
        B_Wq.reshape(D * H, DH), B_Wk.reshape(D * H, DH), B_Wv.reshape(D * H, DH),
        jnp.swapaxes(B_Wo, 1, 2), gate_w.reshape(1, D),
    )
    return out_t.T[None]
```

```python
import functools
import math

import jax
import jax.numpy as jnp
from jax import lax
import jax.experimental.pallas as pl
import jax.experimental.pallas.tpu as pltpu

F32 = jnp.float32
BF16 = jnp.bfloat16
U32 = jnp.uint32

LANES = 128
HALF = LANES // 2
A_HEADS = 16
A_WINDOW = 256
A_GROUP = 4
MASK_VALUE = -1e9
LOG2E = math.log2(math.e)

CHUNK = 512
FOLD_PAIRS = 2

PLAN = dict(a_exp=(1, 0), tail_scores=(10, 0.5), side_scores=(11, 0.5), a_regroup=(14, 0),
            mix=(16, 0), scores=(17, 0), a_scores=(17, 0.5))

HK = (
    (((0, 1, 0), (0, 0, 0), (0, 0, 0)), ((1, -1, 0), (0, 0, 0)), ((1, 1, 0), (0, 0, 0)),
     (1, 0, 0), (1, 1, 0)),
    (((0, 0, 0), (1, 0, 0), (0, 0, 0)), ((0, 0, 0), (-1, 1, 0)), ((0, 0, 0), (1, 1, 0)),
     (0, 1, 0), (1, 1, 0)),
    (((1, -1, 0), (0, 0, 0), (1, 0, 0)), ((1, 0, 0), (-1, 0, 0)), ((1, 0, 0), (0, 0, 0)),
     (1, 0, 0), (1, 0, 0)),
    (((0, 0, 0), (0, 0, 0), (1, 0, 0)), ((1, 0, -1), (-1, 0, 1)), ((0, 0, 0), (1, 0, -1)),
     (1, 0, -1), (-1, 0, 0)),
    (((0, 0, 0), (-1, 1, 0), (0, -1, 0)), ((0, -1, 0), (0, 1, 0)), ((0, 0, 0), (0, 1, 0)),
     (0, 1, 0), (0, 1, 0)),
    (((0, 0, 0), (0, 0, 0), (0, 1, 0)), ((0, 1, 1), (0, -1, -1)), ((0, 1, -1), (0, 0, 0)),
     (0, 1, 1), (0, 1, -1)),
    (((0, 0, 1), (0, 0, 0), (0, 0, 0)), ((1, 0, -1), (0, 0, 0)), ((-1, 0, 1), (-1, 0, 1)),
     (1, 0, -1), (0, 0, 1)),
    (((0, 0, 1), (0, 0, 0), (0, 1, 1)), ((0, 0, 1), (0, 0, 0)), ((0, 0, 1), (0, 0, 0)),
     (0, 0, 1), (0, 0, 1)),
    (((0, 0, 0), (0, 0, 1), (0, 1, 0)), ((0, -1, 0), (0, 1, 1)), ((0, 1, -1), (0, 1, 0)),
     (0, 1, 0), (0, 0, 1)),
    (((1, 0, 1), (1, 0, 0), (0, 0, 0)), ((0, 0, 0), (1, 0, 0)), ((1, 0, 0), (1, 0, 0))),
    (((0, 1, 0), (1, 0, 0), (0, 0, 0)), ((0, 1, 0), (-1, 0, 0)), ((1, 0, 0), (0, -1, 0))),
    (((0, 0, 1), (0, 0, 0), (-1, 0, 0)), ((1, 0, -1), (-1, 0, 0)), ((1, 0, 0), (1, 0, -1))),
    (((0, 1, 0), (0, 1, 1), (0, 0, 0)), ((0, 1, 0), (0, 0, 0)), ((0, 1, 0), (0, 1, 0))),
    (((0, 0, 0), (0, 0, 1), (0, 0, 0)), ((0, 0, 0), (0, 1, 1)), ((0, -1, 1), (0, -1, 1))),
    (((0, 0, 0), (0, 0, -1), (1, 0, 1)), ((0, 0, 0), (0, 0, 1)), ((0, 0, 0), (0, 0, 1))),
)
HK_ROW = 9

_NN = (((1,), (0,)), ((), ()))
_NT = (((1,), (1,)), ((), ()))


def _dot(a, b, dims=_NN):
    return lax.dot_general(a, b, dims, preferred_element_type=F32)


def _pack(x):
    return pltpu.bitcast(x.astype(BF16), U32)


def _halves(words):
    return pltpu.bitcast(words << 16, F32), pltpu.bitcast(words & U32(0xFFFF0000), F32)


def _bf16(words):
    return pltpu.bitcast(words, BF16)


def _transposed(x):
    return pltpu.bitcast(x.T, U32)


def _iota(shape, axis):
    return lax.broadcasted_iota(jnp.int32, shape, axis)


def _rotate(x, shift):
    return pltpu.roll(x, shift % LANES, 1) if shift else x


def _signed_sum(terms):
    terms = [term for term in terms if term[0]]
    sign, total = terms.pop(max(range(len(terms)), key=lambda n: terms[n][0]))
    total = total if sign > 0 else -total
    for sign, x in terms:
        total = total + x if sign > 0 else total - x
    return total


def _weigh(weights, blocks):
    return _signed_sum((w, x) for ws, row in zip(weights, blocks) for w, x in zip(ws, row))


def _shuffle(x, index, axis):
    return jnp.take_along_axis(x, index, axis, mode="promise_in_bounds")


def _skew(xs, dtype):
    n = len(xs)
    zero = jnp.zeros((8, LANES), dtype)
    lane = _iota(zero.shape, 1)
    ys = [xs[-q % n] for q in range(n)]
    k = 1
    while k < n:
        upper = (lane & (k * LANES // n)) != 0
        pairs = [(ys[(q - k) % n], ys[q]) for q in range(n)]
        ys = [None if a is None and b is None else
              jnp.where(upper, zero if a is None else a, zero if b is None else b)
              for a, b in pairs]
        k *= 2
    return [zero if y is None else y for y in ys]


def _kernel(xt_hbm, wqkv_hbm, awo_hbm, mem0_hbm, wq_hbm, wk_hbm, wv_hbm, wot_hbm, gw_hbm,
            out_hbm,
            xt_v, wqkv_v, awo_v, mem0_v, gw_v, wq_v, wk_v, wv_v, wot_v,
            wqkvt_v, awot_v, x_v, q_v, k_v, vt_v, gate_v, w_v, corner_v, low_v,
            mem_v, h_v, tails_v, y_v, pair_v, zu_v, zt_v, s_v, raw_v, e_v, p_v, ot_v, b_v, out_v,
            in_sem, w_sem, out_sem, *, S, D, H, DH, M, SEG):
    L = M + SEG
    NG = L // 8
    DF = D // LANES
    D1 = DF * LANES
    D2 = D - D1
    NP = H // 2
    NQB = S // LANES
    SPB = LANES // SEG
    ADH = D // A_HEADS
    AGW = A_GROUP * ADH
    NAG = A_HEADS // A_GROUP
    AQ = LANES // A_GROUP
    WB = A_WINDOW // LANES

    def group(i):
        return slice(i * 8, (i + 1) * 8)

    def tile(j):
        return slice(j * LANES, (j + 1) * LANES)

    copies = {}

    def fetch(name, src, dst, columns=None):
        if columns:
            columns = pl.ds(columns[0], columns[1] - columns[0])
            src, dst = src.at[:, columns], dst.at[:, columns]
        copies[name] = pltpu.make_async_copy(src, dst, in_sem.at[len(copies)])
        copies[name].start()

    def wait(*names):
        for name in names:
            copies[name].wait()

    def pair_copies(p):
        moves = [(src.bitcast(U32).at[:, p, :], dst.at[p])
                 for src, dst in ((wk_hbm, wk_v), (wq_hbm, wq_v), (wv_hbm, wv_v))]
        moves += [(wot_hbm.at[pl.ds(2 * p, 2)], wot_v.at[pl.ds(2 * p, 2)])]
        return [pltpu.make_async_copy(src, dst, w_sem.at[i * NP + p])
                for i, (src, dst) in enumerate(moves)]

    fetch("gate", gw_hbm, gw_v)
    fetch("wv", wqkv_hbm, wqkv_v, (2 * D, 3 * D))
    fetch("x0", xt_hbm, xt_v, (0, CHUNK))
    fetch("x1", xt_hbm, xt_v, (CHUNK, S - CHUNK))
    fetch("wqk", wqkv_hbm, wqkv_v, (0, 2 * D))
    fetch("x2", xt_hbm, xt_v, (S - CHUNK, S))
    fetch("wo", awo_hbm, awo_v)
    fetch("mem", mem0_hbm, mem0_v)
    for p in range(NP):
        for copy in pair_copies(p):
            copy.start()

    for g in range(NAG):
        k_v[g, :A_WINDOW // 2] = _pack(
            jnp.where(_iota((A_WINDOW, LANES), 1) == AGW, MASK_VALUE, 0.0))
        for kb in range(WB):
            vt_v[g, kb] = jnp.zeros((HALF, LANES), U32)
    ot_v[1] = jnp.zeros(ot_v.shape[1:], U32)
    b_v[1] = jnp.zeros(b_v.shape[1:], F32)

    head_rows = [(j * ADH // 8 * 8, -(-(j + 1) * ADH // 8) * 8) for j in range(A_GROUP)]

    def merge_heads(parts):
        tiles = []
        for r in range(0, AGW, 8):
            own = [(j, parts[j][r - lo:r - lo + 8])
                   for j, (lo, hi) in enumerate(head_rows) if lo <= r < hi]
            tiles.append(own[0][1] if len(own) == 1 else jnp.where(
                _iota((8, LANES), 0) < own[1][0] * ADH - r, own[0][1], own[1][1]))
        return jnp.concatenate(tiles, 0)

    def split_heads(x, fill):
        parts = []
        for j, (lo, hi) in enumerate(head_rows):
            row = _iota((hi - lo, x.shape[1]), 0) + lo
            parts.append(jnp.where((row >= j * ADH) & (row < (j + 1) * ADH), x[lo:hi], fill))
        return jnp.concatenate(parts, 0)

    def transpose_wqkv(lo, hi):
        for c in range(lo, hi, LANES):
            n = min(LANES, hi - c)
            wqkvt_v[c:c + n, :] = wqkv_v[:, c:c + n].T

    def project_a(part, c, g, extra=0):
        row = part * D + g * AGW
        r = _dot(wqkvt_v[row:row + AGW + extra, :], xt_v[:, c * CHUNK:(c + 1) * CHUNK])
        return [(c * CHUNK // LANES + t, r[:, tile(t)]) for t in range(CHUNK // LANES)]

    def project_q(c, g):
        word = _iota((AGW // 2, LANES), 0)
        owner = functools.reduce(jnp.add, [(word >= j * ADH // 2).astype(jnp.int32)
                                           for j in range(1, A_GROUP)])
        quarter = ((_iota(word.shape, 1) >> (AQ.bit_length() - 1)) - owner) & (A_GROUP - 1)
        bias = _pack(jnp.where(_iota((LANES - AGW, LANES), 0) == 0, 1.0, 0.0))
        for qb, r in project_a(0, c, g):
            r = r * (ADH ** -0.5 * LOG2E)
            q = _pack(merge_heads([_rotate(r[lo:hi], j * AQ)
                                   for j, (lo, hi) in enumerate(head_rows)]))
            for u in range(A_GROUP):
                q_v[qb, g, u] = jnp.concatenate([jnp.where(quarter == u, q, U32(0)), bias], 0)
        cols = slice(c * CHUNK, (c + 1) * CHUNK)
        xt = xt_v[tile(g), cols] if g < DF else jnp.concatenate([xt_v[D1:, cols]] * 2, 0)
        x_v[c * CHUNK // 2:(c + 1) * CHUNK // 2, tile(g)] = _transposed(xt)

    def project_k(c, g):
        for qb, r in project_a(1, c, g):
            keys = jnp.concatenate([r, jnp.zeros((LANES - AGW, LANES), F32)], 0).T
            row = (A_WINDOW + qb * LANES) // 2
            k_v[g, row:row + HALF] = _pack(keys)

    def project_v(c, g):
        extra = 16 if g == NAG - 1 else 0
        for qb, r in project_a(2, c, g, extra):
            vt_v[g, WB + qb] = _pack(split_heads(r[:AGW], 1.0))
            if extra:
                gate_v[qb] = jax.nn.sigmoid(r[AGW:AGW + 8])

    chunks = S // CHUNK
    wait("gate", "wv", "x0")
    transpose_wqkv(2 * D, 3 * D)
    wqkvt_v[3 * D:] = jnp.broadcast_to(gw_v[...].astype(F32)[None], (16, D)).astype(BF16)
    for c in range(chunks - 1):
        if c == 1:
            wait("x1")
        for g in reversed(range(NAG)):
            project_v(c, g)
    wait("wqk", "x2", "wo", "mem")
    project_v(chunks - 1, NAG - 1)
    transpose_wqkv(0, 2 * D)
    mem_v[...] = jnp.concatenate([mem0_v[...].astype(F32), jnp.zeros((M, LANES - D2), F32)], 1)
    for g in range(NAG):
        rows = split_heads(awo_v[g * AGW:(g + 1) * AGW, :].astype(F32), 0.0)
        awot_v[g] = _transposed(rows.astype(BF16))
    for c in range(chunks):
        for g in range(NAG):
            project_q(c, g)
            project_k(c, g)
    for g in range(NAG - 1):
        project_v(chunks - 1, g)

    sixteens = [k * LANES + r for r in range(0, LANES, 16) for k in range(DF)]
    sixteens += list(range(D1, D, 16))

    def reorder(x):
        return jnp.concatenate([x[r:r + 16] for r in sixteens], 0)

    def rows16(x, r):
        n = sixteens.index(r) * 16
        return x[n:n + 16]

    def store_triple(n, p, panels):
        blocks = [[jnp.concatenate([panel(k * LANES + r) for r in range(0, LANES, 16)], 0)
                   for panel in panels] for k in range(DF)]
        for m, (weights, *_) in enumerate(HK):
            w_v[n, p, m] = _pack(_weigh(weights, blocks))

    def fold(p, i, lhs, rhs, scale):
        side = jnp.concatenate([_dot(rhs[e][D1:], lhs[e], _NT) * scale for e in range(2)], 0).T
        corner_v[i, p] = _pack(jnp.concatenate(
            [side[D1:], jnp.zeros((LANES - D2, LANES), F32)], 0))
        low = []
        for e in range(2):
            r = _dot(lhs[e], rhs[e][:D1], _NT) * scale
            store_triple(2 * i + e, p, [functools.partial(rows16, r[:, tile(j)])
                                        for j in range(DF)])
            low.append(r[D1:])
        return functools.partial(rows16, side), jnp.concatenate(low, 0)

    @pl.loop(0, NP, step=FOLD_PAIRS)
    def fold_pairs(start):
        pairs = [start + n for n in range(FOLD_PAIRS)]
        for p in pairs:
            for copy in pair_copies(p):
                copy.wait()
        for p in pairs:
            wq = [w.astype(BF16) for w in _halves(wq_v[p])]
            wk, wv = ([reorder(w).astype(BF16) for w in _halves(ref[p])] for ref in (wk_v, wv_v))
            key_side, key_low = fold(p, 0, wk, wq, DH ** -0.5 * LOG2E)
            val_side, val_low = fold(p, 1, wv, [wot_v[2 * p], wot_v[2 * p + 1]], 1.0)
            query = key_low.T
            store_triple(4, p, [key_side, val_side, lambda r: query[r:r + 16]])
            low_v[pl.ds(pl.multiple_of(p * HALF, HALF), HALF), :] = _pack(val_low)

    def older():
        return _iota((AQ, LANES), 0) > (_iota((AQ, LANES), 1) & (AQ - 1))

    def a_scores(qb, g, u):
        start = (qb * LANES + u * AQ) // 2
        if not isinstance(start, int):
            start = pl.multiple_of(start, AQ // 2)
        part = (A_WINDOW + AQ) // 6
        q = _bf16(q_v[qb, g, u])
        s = jnp.concatenate([_dot(_bf16(k_v[g, pl.ds(start + n * part, part), :]), q)
                             for n in range(3)], 0)
        s = jnp.concatenate([jnp.where(older(), s[:AQ], s[A_WINDOW:]), s[AQ:A_WINDOW]], 0)
        raw_v[u, :A_WINDOW] = s
        raw_v[u, A_WINDOW:] = jnp.broadcast_to(jnp.max(s, 0, keepdims=True), (8, LANES))

    def a_exp(u):
        e = jnp.exp2(raw_v[u, :A_WINDOW]
                     - jnp.concatenate([raw_v[u, A_WINDOW:]] * (A_WINDOW // 8), 0))
        e_v[u] = _pack(jnp.concatenate(
            [jnp.where(older(), e[:AQ], 0.0), e[AQ:], jnp.where(older(), 0.0, e[:AQ])], 0))

    def a_regroup():
        for r in range(0, A_WINDOW + LANES, 16):
            tiles = [e_v[u, (r - u * AQ) // 2:(r - u * AQ) // 2 + 8]
                     if 0 <= r - u * AQ < A_WINDOW + AQ else None for u in range(A_GROUP)]
            for j, words in enumerate(_skew(tiles, U32)):
                p_v[j, r // 2:r // 2 + 8] = words

    def a_values(qb, g, slot):
        for j, (lo, _) in enumerate(head_rows):
            values = jnp.concatenate(
                [vt_v[g, qb + kb, j * AQ // 2:(j + 1) * AQ // 2] for kb in range(WB + 1)], 1)
            o = _dot(_bf16(values), _bf16(p_v[j]))
            ones = 0 if lo < j * ADH else AQ - 1
            o = o * (1.0 / o[ones:ones + 1])
            row = (g * LANES + j * AQ) // 2
            ot_v[slot, row:row + AQ // 2] = _rotate(_pack(o), -j * AQ)

    def mix(qb, slot, j):
        n = LANES if j < DF else D2
        wo = jnp.concatenate([awot_v[g, j * HALF:j * HALF + n // 2] for g in range(NAG)], 1)
        a = _dot(_bf16(wo), _bf16(ot_v[slot]))
        b = b_v[slot, :, tile(j)].T
        if j == DF:
            b = b[:D2] + b[D2:]
        gate = gate_v[qb][0:1]
        out_v[qb, j * LANES:j * LANES + n, :] = (gate * a + (1.0 - gate) * b).astype(BF16)

    def key_groups(i):
        return NG if i == 0 else i + 1

    def query_groups(g):
        return [i for i in range(NG) if g < key_groups(i)]

    def pair_rows(even, odd):
        rows = jnp.concatenate([x[group(g)] for g in range(NG) for x in (even, odd)], 0)
        return _pack(rows).reshape(NG, 8, LANES)

    def split_pair(x):
        low = _iota(x.shape, 1) < D2
        return pair_rows(jnp.where(low, x, 0.0), jnp.where(low, 0.0, x))

    def load_rows(qb, t):
        tail = mem_v[:, D1:]
        h_v[:M, :D1] = mem_v[:, :D1]
        h_v[:M, D1:] = tail + _rotate(tail, D2)
        row = pl.multiple_of((qb * LANES + t * SEG) // 2, 8)
        h_v[M:] = _bf16(x_v[pl.ds(row, SEG // 2), :]).astype(F32)
        tails_v[...] = split_pair(h_v[:, D1:])

        def blocks(x, start, n):
            return [x[start:start + n, tile(k)] for k in range(DF)]

        h = h_v[:, :D1]
        for r, (_, weights, _, row_weights, _) in enumerate(HK[:HK_ROW]):
            w_v[5, 0, r, :SEG] = pltpu.bitcast(jnp.concatenate(
                [_weigh([row_weights], [blocks(h, 0, L - 16)]),
                 _weigh(weights, [blocks(h, L - 16, 8), blocks(h, L - 8, 8)])], 0), U32)
        for n in range(SPB if t == 0 else 0):
            row = pl.multiple_of((qb * LANES + (n + 1) * SEG - 16) // 2, 8)
            x = _bf16(x_v[pl.ds(row, 8), :D1]).astype(F32)
            for r in range(HK_ROW, len(HK)):
                w_v[5, 0, r, group(n)] = pltpu.bitcast(
                    _weigh(HK[r][1], [blocks(x, 0, 8), blocks(x, 8, 8)]), U32)

    def triples(ns, p, t):
        def products(rs):
            lhs = [pltpu.bitcast(w_v[5, 0, r, :SEG], F32) for r in rs]
            return zip(ns, zip(*[[_dot(x, _bf16(w_v[n, p, r])) for n in ns]
                                 for r, x in zip(rs, lhs)]))

        if t == 0:
            for n, prods in products(range(HK_ROW, len(HK))):
                for m in range(2):
                    for c in range(DF):
                        w_v[n, p, len(HK) + c, m * SEG:(m + 1) * SEG] = pltpu.bitcast(_signed_sum(
                            (hk[2][m][c], x) for hk, x in zip(HK[HK_ROW:], prods)), U32)
        results = []
        for n, prods in products(range(HK_ROW)):
            rows, last = [x[:-8] for x in prods], [x[-8:] for x in prods]
            results.append([jnp.concatenate(
                [_signed_sum((hk[4][c], x) for hk, x in zip(HK, rows))]
                + [_signed_sum(
                    [(1, pltpu.bitcast(w_v[n, p, len(HK) + c, group(m * SPB + t)], F32))]
                    + [(hk[2][m][c], x) for hk, x in zip(HK, last)]) for m in range(2)], 0)
                for c in range(DF)])
        return results

    def project(i, p, t, done):
        even, odd = triples([2 * i, 2 * i + 1], p, t)
        done(even[0][:8])
        for j in range(DF):
            zu_v[i, j, :, group(p)] = pair_rows(even[j], odd[j])

    def project_tail(p, t, done):
        panels, = triples([4], p, t)
        done(panels[0][:8])
        for i in range(2):
            zu_v[i, DF, :, group(p)] = split_pair(
                panels[i] + _dot(h_v[:, D1:], _bf16(corner_v[i, p])))
        y_v[:, group(p)] = split_pair(panels[2])

    started = set()

    def add_scores(i, g, s):
        s_v[g, group(i)] = s_v[g, group(i)] + s if (i, g) in started else s
        started.add((i, g))

    def tail_scores(i):
        s = _dot(h_v[:key_groups(i) * 8, D1:], _bf16(zt_v[DF + 1, i]))
        sub, lane = _iota((8, LANES), 0), _iota((8, LANES), 1)
        for g in range(key_groups(i)):
            x = _shuffle(s[group(g)], lane ^ sub, 1)
            x = _shuffle(x, sub ^ (lane & 7), 0)
            add_scores(i, g, _shuffle(x, lane ^ sub, 1))

    def scores(j, g):
        rows = query_groups(g)
        s = _dot(jnp.concatenate([h_v[group(i), tile(j)] for i in rows], 0), _bf16(zt_v[j, g]))
        for n, i in enumerate(rows):
            add_scores(i, g, s[group(n)])

    def softmax():
        sub, lane = _iota((8, LANES), 0), _iota((8, LANES), 1)

        def reduce_keys(tiles, op):
            xs = [functools.reduce(op, row) for row in tiles]
            for k in (1, 2, 4):
                xs = [op(x, _shuffle(x, lane ^ k, 1)) for x in xs]
            return xs

        tiles = [[s_v[g, group(i)] for g in range(key_groups(i))] for i in range(NG)]
        for i in range(1, NG):
            tiles[i][i] = jnp.where((lane & 7) <= sub, tiles[i][i], MASK_VALUE)
        tiles = [[jnp.exp2(x - peak) for x in row]
                 for row, peak in zip(tiles, reduce_keys(tiles, jnp.maximum))]
        for i, (row, total) in enumerate(zip(tiles, reduce_keys(tiles, jnp.add))):
            row = [x * (1.0 / total) for x in row]
            for g, x in enumerate(row):
                s_v[g, group(i)] = x
            row = [_rotate(x, 16 * g) for g, x in enumerate(row)]
            for p, x in enumerate(_skew(row + [None] * (NP - len(row)), F32)):
                pair_v[0, p, group(i)] = x

    def tail_values(p):
        zero = jnp.zeros((8, LANES), U32)
        tails = [tails_v[(b - p) % NP] if (b - p) % NP < NG else zero for b in range(NP)]
        pair_v[1, p] = _dot(pair_v[0, p], _bf16(jnp.concatenate(tails, 0)))

    def values(slot, t):
        for j in (0, 1, DF, 2):
            o = [None] * NG
            for g in range(NG):
                rows = query_groups(g)
                r = _dot(jnp.concatenate([s_v[g, group(i)] for i in rows], 0),
                         _bf16(zu_v[1, j, g]))
                for n, i in enumerate(rows):
                    o[i] = r[group(n)] if o[i] is None else o[i] + r[group(n)]
            o = jnp.concatenate(o, 0)
            if j < DF:
                o += _dot(jnp.concatenate([pair_v[1, p] for p in range(NP)], 1),
                          _bf16(low_v[:, tile(j)]))
            mem_v[:, tile(j)] = o[:M]
            b_v[slot, t * SEG:(t + 1) * SEG, tile(j)] = o[M:]

    def segment(qb, t):
        slot, prev = qb % 2, jnp.maximum(qb - 1, 0)

        def due(task, n, count=1):
            start, stride = PLAN[task]
            return [k for k in range(count) if int(start + k * stride) == n]

        def fence(spare, value=None):
            spare[slot, :8] = jnp.zeros((8, LANES), spare.dtype) if value is None else value

        load_rows(qb, t)
        fence(w_v.at[5, 1])
        started.clear()
        for n in range(3 * NP):
            phase, p = divmod(n, NP)
            for u in due("a_scores", n, A_GROUP):
                a_scores(qb if t < SPB - 1 else jnp.minimum(qb + 1, NQB - 1), (t + 1) % SPB, u)
            exps = due("a_exp", n, A_GROUP)

            def done(x):
                if exps:
                    fence(raw_v.at[pl.ds(A_GROUP, 2)], x)

            if phase:
                project(phase - 1, p, t, done)
            else:
                project_tail(p, t, done)
            for u in exps:
                a_exp(u)
            if due("a_regroup", n):
                fence(e_v.at[pl.ds(A_GROUP, 2)])
                a_regroup()
            for g in range(NG if p == NP - 1 else 0):
                if phase == 0:
                    zt_v[DF + 1, g] = _transposed(_bf16(y_v[g]))
                for j in ([DF], range(DF), [])[phase]:
                    zt_v[j, g] = _transposed(_bf16(zu_v[0, j, g]))
            for i in due("tail_scores", n, NG):
                tail_scores(i)
            for g in due("side_scores", n, NG):
                scores(DF, g)
            if due("scores", n):
                for j in range(DF):
                    for g in range(NG):
                        scores(j, g)
                softmax()
            if due("mix", n) and t == SPB - 1:
                mix(prev, 1 - slot, t)
        fence(zu_v.at[2, 0])
        for p in range(NP):
            tail_values(p)
        fence(pair_v.at[2])
        a_values(qb, t, slot)
        values(slot, t)
        if t < SPB - 1:
            mix(prev, 1 - slot, t)

    def out_copy(qb):
        cols = pl.ds(pl.multiple_of(qb * LANES, LANES), LANES)
        return pltpu.make_async_copy(out_v.at[qb], out_hbm.at[:, cols], out_sem)

    for u in range(A_GROUP):
        a_scores(0, 0, u)

    @pl.loop(0, NQB)
    def token_block(qb):
        for t in range(SPB):
            segment(qb, t)

        @pl.when(qb > 0)
        def _():
            out_copy(qb - 1).start()

    for j in range(DF + 1):
        mix(NQB - 1, (NQB - 1) % 2, j)
    out_copy(NQB - 1).start()
    for qb in range(NQB):
        out_copy(qb).wait()


@functools.partial(jax.jit, static_argnames=("B_seg_len",))
def pallas_gated_mix__sliding_block__memory_aug_recurrent_mem_tr__prompt_kernel(
    A_x, A_wqkv, A_wo, B_x, B_mem0, B_Wq, B_Wk, B_Wv, B_Wo, B_seg_len, gate_w,
):
    del B_x
    batch, S, D = A_x.shape
    _, H, DH = B_Wq.shape
    M, SEG = B_mem0.shape[1], int(B_seg_len)
    L = M + SEG
    DF = D // LANES
    DP = (DF + 1) * LANES
    NP, NG, NQB, NAG = H // 2, L // 8, S // LANES, A_HEADS // A_GROUP
    assert (batch, D, H, M, SEG) == (1, 448, 16, 8, 32) and S % CHUNK == 0

    hbm = pl.BlockSpec(memory_space=pltpu.HBM)
    vmem = pltpu.VMEM
    out_t = pl.pallas_call(
        functools.partial(_kernel, S=S, D=D, H=H, DH=DH, M=M, SEG=SEG),
        out_shape=jax.ShapeDtypeStruct((D, S), A_x.dtype),
        in_specs=[hbm] * 9,
        out_specs=hbm,
        scratch_shapes=[
            vmem((D, S), BF16),
            vmem((D, 3 * D), BF16),
            vmem((D, D), BF16),
            vmem((M, D), BF16),
            vmem((D,), BF16),
            vmem((NP, D, DH), U32),
            vmem((NP, D, DH), U32),
            vmem((NP, D, DH), U32),
            vmem((H, D, DH), BF16),
            vmem((3 * D + 16, D), BF16),
            vmem((NAG, D // 2, LANES), U32),
            vmem((S // 2, DP), U32),
            vmem((NQB, NAG, A_GROUP, HALF, LANES), U32),
            vmem((NAG, (A_WINDOW + S) // 2, LANES), U32),
            vmem((NAG, A_WINDOW // LANES + NQB, HALF, LANES), U32),
            vmem((NQB, 8, LANES), F32),
            vmem((6, NP, len(HK) + DF, HALF, LANES), U32),
            vmem((2, NP, HALF, LANES), U32),
            vmem((NP * HALF, DF * LANES), U32),
            vmem((M, DP), F32),
            vmem((L, DP), F32),
            vmem((NG, 8, LANES), U32),
            vmem((NG, HALF, LANES), U32),
            vmem((3, NP, L, LANES), F32),
            vmem((3, DF + 1, NG, HALF, LANES), U32),
            vmem((DF + 2, NG, HALF, LANES), U32),
            vmem((NG, L, LANES), F32),
            vmem((A_GROUP + 2, A_WINDOW + 8, LANES), F32),
            vmem((A_GROUP + 2, (A_WINDOW + LANES // A_GROUP) // 2, LANES), U32),
            vmem((A_GROUP, (A_WINDOW + LANES) // 2, LANES), U32),
            vmem((2, NAG * HALF, LANES), U32),
            vmem((2, LANES, DP), F32),
            vmem((NQB, D, LANES), BF16),
            pltpu.SemaphoreType.DMA((8,)),
            pltpu.SemaphoreType.DMA((4 * NP,)),
            pltpu.SemaphoreType.DMA(()),
        ],
        compiler_params=pltpu.CompilerParams(vmem_limit_bytes=100 * 1024 * 1024),
    )(
        A_x[0].T, A_wqkv, A_wo, B_mem0[0], B_Wq, B_Wk, B_Wv,
        jnp.swapaxes(B_Wo, 1, 2), gate_w,
    )
    return out_t.T[None]
```
